```python
import os as _os
_os.environ.setdefault('JAX_PLATFORMS', 'cpu')
import jax
import jax.numpy as jnp

def _softmax(x, axis=-1):
    return jax.nn.softmax(x, axis=axis)

def _gelu(x):
    return jax.nn.gelu(x, approximate=True)

def _silu(x):
    return jax.nn.silu(x)

def _sigmoid(x):
    return jax.nn.sigmoid(x)

def _layernorm(x, axis=-1, eps=1e-05):
    m = jnp.mean(x, axis=axis, keepdims=True)
    v = jnp.var(x, axis=axis, keepdims=True)
    return (x - m) / jnp.sqrt(v + eps)

def _scatter_add(tgt, idx, src, axis=0):
    return tgt.at[idx].add(src)

def _segment_sum(src, seg, n):
    return jax.ops.segment_sum(src, seg, n)

class _Rng:

    def __init__(self, key):
        self._k = key

    def _next(self):
        self._k, sub = jax.random.split(self._k)
        return sub

    def normal(self, shape):
        return jax.random.normal(self._next(), shape, dtype=jnp.bfloat16)

    def randint(self, lo, hi, shape):
        return jax.random.randint(self._next(), shape, lo, hi, dtype=jnp.int32)

    def uniform(self, shape, lo=0.0, hi=1.0):
        return jax.random.uniform(self._next(), shape, jnp.bfloat16, lo, hi)

    def permutation(self, n):
        return jax.random.permutation(self._next(), n)
kernel_name = 'standalone__conformer_conv_module__speech'

def setup_inputs():
    _rng = _Rng(jax.random.key(int.from_bytes(__import__("os").urandom(4), "little")))
    _w = lambda a: (lambda t: t.astype(jnp.bfloat16) if jnp.issubdtype(t.dtype, jnp.floating) else t)(jnp.asarray(a))
    B, T, D, K = (2, 4000, 512, 15)
    return {'x': _w((lambda *s: _rng.normal(s) * 0.2)(B, T, D)), 'w_pw1': _w((lambda *s: _rng.normal(s) * 0.2)(D, 2 * D)), 'dw': _w((lambda *s: _rng.normal(s) * 0.05)(K, D)), 'w_pw2': _w((lambda *s: _rng.normal(s) * 0.05)(D, D))}

def reference(x, w_pw1, dw, w_pw2):
    B, T, D = x.shape
    K = dw.shape[0]
    h = x @ w_pw1
    a, b = (h[..., :D].copy(), h[..., D:].copy())
    h = a * _sigmoid(b)
    pad = K // 2
    hp = jnp.pad(h, ((0, 0), (pad, pad), (0, 0)))
    out = jnp.zeros_like(h)
    for i in range(K):
        out = out + hp[:, i:i + T, :] * dw[i][None, None, :]
    return _silu(out) @ w_pw2
```

```python
import functools
import jax
import jax.numpy as jnp
import jax.experimental.pallas as pl
import jax.experimental.pallas.tpu as pltpu

LC = 128
H = 8
LEAD = 16
A_ROWS = 240
SEG = 800
NSEG = 3
L = SEG * NSEG
F32 = jnp.float32
PIECES = (1200, 640, 320, 240)


def kernel(x_hbm, w1_hbm, dw_hbm, w2_hbm, o_hbm,
           x_v, w1_v, dw_v, w2_v, ga_v, gb_v, s_v, o_v, sem_i, sem_o, *, B, T, D, K):
    nC = D // LC
    R = B * T
    pad = K // 2
    n_it = (R - SEG) // L
    assert SEG + n_it * L == R and T % SEG == 0
    GB = H + (L - SEG) + LEAD
    bnd_it = [(b * T - 2 * SEG) // L for b in range(1, B)]
    for b in range(1, B):
        assert (b * T - 2 * SEG) % L == 0

    xb = [0, A_ROWS + LEAD, SEG + LEAD, SEG + L + LEAD, R]

    def x_copy(q):
        lo, hi = xb[q], xb[q + 1]
        return pltpu.make_async_copy(x_hbm.at[lo:hi], x_v.at[lo:hi], sem_i.at[q])

    w1_copy = pltpu.make_async_copy(w1_hbm, w1_v, sem_i.at[4])
    dw_copy = pltpu.make_async_copy(dw_hbm, dw_v, sem_i.at[5])
    w2_copy = pltpu.make_async_copy(w2_hbm, w2_v, sem_i.at[6])

    x_copy(0).start()
    w1_copy.start()
    dw_copy.start()
    x_copy(1).start()
    w2_copy.start()
    x_copy(2).start()
    x_copy(3).start()

    x_v[R:R + LEAD, :] = jnp.zeros((LEAD, D), x_v.dtype)
    P0 = GB - (SEG + LEAD + H)
    for c in range(nC):
        gb_v[c, P0:P0 + H, :] = jnp.zeros((H, LC), F32)

    def glu(xv, c):
        a = jnp.dot(xv, w1_v[:, c * LC:(c + 1) * LC], preferred_element_type=F32)
        b = jnp.dot(xv, w1_v[:, D + c * LC:D + (c + 1) * LC], preferred_element_type=F32)
        return a * jnp.tanh(0.5 * b) + a

    def conv(g_ref, c, first, m):
        dwf = dw_v[:, c * LC:(c + 1) * LC].astype(F32) * 0.25
        acc = None
        for k in range(K):
            o = first - pad + k
            term = g_ref[c, o:o + m, :] * dwf[k:k + 1, :]
            acc = term if acc is None else acc + term
        return acc * jnp.tanh(acc) + acc

    def pw2_out(s, r0, pieces):
        off = 0
        for p in pieces:
            rows = pl.ds(r0 + off, p)
            o_v[rows, :] = jnp.dot(s[off:off + p], w2_v[...], preferred_element_type=F32).astype(o_v.dtype)
            pltpu.make_async_copy(o_v.at[rows], o_hbm.at[rows], sem_o).start()
            off += p

    x_copy(0).wait()
    w1_copy.wait()
    dw_copy.wait()
    xv = x_v[0:A_ROWS + LEAD, :]
    for c in range(nC):
        gb_v[c, P0 + H:P0 + H + A_ROWS + LEAD, :] = glu(xv, c)
    s0 = jnp.concatenate([conv(gb_v, c, P0 + H, A_ROWS) for c in range(nC)], axis=1)
    s_v[...] = s0

    x_copy(1).wait()
    w2_copy.wait()
    xv = x_v[A_ROWS + LEAD:SEG + LEAD, :]
    for c in range(nC):
        gb_v[c, P0 + H + A_ROWS + LEAD:GB, :] = glu(xv, c)
    s1 = jnp.concatenate([conv(gb_v, c, P0 + H + A_ROWS, SEG - A_ROWS) for c in range(nC)], axis=1)
    s = jnp.concatenate([s_v[...], s1], axis=0).astype(jnp.bfloat16)
    pw2_out(s, 0, (SEG,))

    x_copy(2).wait()

    def body(i, carry):
        @pl.when(i == 1)
        def _():
            x_copy(3).wait()
        r0 = pl.multiple_of(SEG + i * L, 16)
        keep = i != bnd_it[0]
        for c in range(nC):
            ga_v[c, 0:H + LEAD, :] = gb_v[c, GB - (H + LEAD):GB, :]
        xv = x_v[pl.ds(r0 + LEAD, L), :]
        n0 = SEG - LEAD
        for c in range(nC):
            g = glu(xv, c)
            ga_v[c, H + LEAD:H + SEG, :] = g[0:n0]
            ga_v[c, H + SEG:H + SEG + H, :] = jnp.where(keep, g[n0:n0 + H], 0.0)
            gb_v[c, 0:H, :] = jnp.where(keep, g[n0 - H:n0], 0.0)
            gb_v[c, H:GB, :] = g[n0:]
        ss = []
        for c in range(nC):
            ss.append(jnp.concatenate([conv(ga_v, c, H, SEG), conv(gb_v, c, H, L - SEG)], axis=0))
        s = jnp.concatenate(ss, axis=1).astype(jnp.bfloat16)
        pw2_out(s, r0, PIECES)
        return carry

    jax.lax.fori_loop(0, n_it, body, 0)
    pltpu.make_async_copy(o_v, o_hbm, sem_o).wait()


@jax.jit
def pallas_standalone__conformer_conv_module__speech_kernel(x, w_pw1, dw, w_pw2):
    B, T, D = x.shape
    K = dw.shape[0]
    R = B * T
    nC = D // LC
    out = pl.pallas_call(
        functools.partial(kernel, B=B, T=T, D=D, K=K),
        in_specs=[pl.BlockSpec(memory_space=pl.ANY)] * 4,
        out_specs=pl.BlockSpec(memory_space=pl.ANY),
        out_shape=jax.ShapeDtypeStruct((R, D), x.dtype),
        scratch_shapes=[
            pltpu.VMEM((R + LEAD, D), x.dtype),
            pltpu.VMEM((D, 2 * D), w_pw1.dtype),
            pltpu.VMEM((K, D), dw.dtype),
            pltpu.VMEM((D, D), w_pw2.dtype),
            pltpu.VMEM((nC, H + SEG + H, LC), F32),
            pltpu.VMEM((nC, H + (L - SEG) + LEAD, LC), F32),
            pltpu.VMEM((A_ROWS, D), F32),
            pltpu.VMEM((R, D), x.dtype),
            pltpu.SemaphoreType.DMA((7,)),
            pltpu.SemaphoreType.DMA(()),
        ],
        compiler_params=pltpu.CompilerParams(vmem_limit_bytes=100 * 1024 * 1024,
                                             disable_bounds_checks=True, disable_semaphore_checks=True),
    )(x.reshape(R, D), w_pw1, dw, w_pw2)
    return out.reshape(B, T, D)
```

```python
import functools

import jax
import jax.numpy as jnp
import jax.experimental.pallas as pl
import jax.experimental.pallas.tpu as pltpu

LC = 128
H = 8
LEAD = 16
P2 = 464
XB = P2 + LEAD
XP = 2 * XB
RAMP = (
    ((0, 416, 0, 1, 0),),
    ((416, XP, 0, 1, 0), (0, XP, 0, 1, 1)),
    ((0, XB, 1, 3, 0), (XB, XP, 1, 2, 0), (0, XP, 1, 2, 1)),
    ((0, XB, 3, 4, 0), (0, XB, 2, 4, 1), (XB, XP, 2, 4, 0), (XB, XP, 2, 4, 1)),
)
PRO_PIECES = (464, 272, 192)
TAIL_PIECES = (1440, 480, 160)
F32 = jnp.float32
BF16 = jnp.bfloat16


def _kernel(x_hbm, w1_hbm, dw_hbm, w2_hbm, o_hbm,
            x_v, w1_v, dw_v, w2_v, gp_v, g_v, h_v, o_v, sem_i, sem_o, *, B, T, D, K):
    nC = D // LC
    pad = K // 2
    assert B == 2 and nC == 4 and pad <= H
    LX = T - XB
    LO = T - P2
    GP = H + XB
    nR = len(RAMP)
    halves = ((0, nC, 1, nC + 1), (2, nC + 2, 3, nC + 3))

    def x_head_copies(lo, hi, c, s):
        out = []
        for b in range(B):
            l, h = max(lo, b * XB), min(hi, (b + 1) * XB)
            if l < h:
                out.append(pltpu.make_async_copy(
                    x_hbm.at[b * T + l - b * XB:b * T + h - b * XB, c * LC:(c + 1) * LC],
                    x_v.at[c, l:h], sem_i.at[s]))
        return out

    def w1_copy(k0, k1, t, s):
        return pltpu.make_async_copy(w1_hbm.at[k0 * LC:k1 * LC, t * LC:(t + 1) * LC],
                                     w1_v.at[t, k0 * LC:k1 * LC], sem_i.at[s])

    grp = []
    x_have = [0] * nC
    w_have = [0, 0]
    for q, blk in enumerate(RAMP):
        cps = []
        for (lo, hi, k0, k1, hf) in blk:
            for k in range(k0, k1):
                if x_have[k] < hi:
                    cps += x_head_copies(x_have[k], hi, k, q)
                    x_have[k] = hi
            if w_have[hf] < k1:
                cps += [w1_copy(w_have[hf], k1, t, q) for t in halves[hf]]
                w_have[hf] = k1
        if q == nR - 1:
            cps.append(pltpu.make_async_copy(dw_hbm, dw_v, sem_i.at[q]))
            cps += [pltpu.make_async_copy(w2_hbm.at[:, n * LC:(n + 1) * LC], w2_v.at[n], sem_i.at[q])
                    for n in range(nC)]
        grp.append(cps)
    assert x_have == [XP] * nC and w_have == [nC, nC]
    for b in range(B):
        grp.append([pltpu.make_async_copy(x_hbm.at[b * T + XB:(b + 1) * T, c * LC:(c + 1) * LC],
                                          x_v.at[c, XP + b * LX:XP + (b + 1) * LX], sem_i.at[nR + b])
                    for c in range(nC)])
    for cps in grp:
        for cp in cps:
            cp.start()

    def wait(q):
        for cp in grp[q]:
            cp.wait()

    zeros = jnp.zeros((H, LC), F32)
    for c in range(nC):
        for b in range(B):
            gp_v[c, b * GP:b * GP + H, :] = zeros
        g_v[c, H + LO:H + LO + H, :] = zeros

    def load_x(rows, k0=0, k1=nC):
        parts = [x_v[c, rows, :] for c in range(k0, k1)]
        return parts[0] if len(parts) == 1 else jnp.concatenate(parts, axis=1)

    def mm1(xv, t):
        return jnp.dot(xv, w1_v[t], preferred_element_type=F32)

    def gate(a, b):
        return a * jnp.tanh(0.5 * b) + a

    def conv(g_ref, c, first, m):
        dwf = dw_v[:, c * LC:(c + 1) * LC].astype(F32) * 0.25
        acc = None
        for k in range(K):
            o = first - pad + k
            term = g_ref[c, o:o + m, :] * dwf[k:k + 1, :]
            acc = term if acc is None else acc + term
        return acc * jnp.tanh(acc) + acc

    def out_start(n, v0, h0, m):
        pltpu.make_async_copy(o_v.at[n, pl.ds(v0, m)], o_hbm.at[pl.ds(h0, m), n * LC:(n + 1) * LC], sem_o).start()

    def pw2_out(s, v0, pieces, h0=None):
        off = 0
        for p in pieces:
            sp = s[off:off + p].astype(BF16)
            for n in range(nC):
                o_v[n, pl.ds(v0 + off, p), :] = jnp.dot(sp, w2_v[n], preferred_element_type=F32).astype(o_v.dtype)
                if h0 is not None:
                    out_start(n, v0 + off, h0 + off, p)
            off += p

    def prologue():
        for q, blk in enumerate(RAMP):
            wait(q)
            for (lo, hi, k0, k1, hf) in blk:
                xv = load_x(slice(lo, hi), k0, k1)
                wv = jnp.concatenate([w1_v[t, k0 * LC:k1 * LC, :] for t in halves[hf]], axis=1)
                part = jnp.dot(xv, wv, preferred_element_type=F32)
                if k0 > 0:
                    part = part + h_v[hf, lo:hi, :]
                if k1 < nC:
                    h_v[hf, lo:hi, :] = part
                else:
                    for j in range(2):
                        g = gate(part[:, 2 * j * LC:(2 * j + 1) * LC], part[:, (2 * j + 1) * LC:(2 * j + 2) * LC])
                        for b in range(B):
                            l, h = max(lo, b * XB), min(hi, (b + 1) * XB)
                            if l < h:
                                o = b * GP + H - b * XB
                                gp_v[2 * hf + j, o + l:o + h, :] = g[l - lo:h - lo]
        s = jnp.concatenate(
            [jnp.concatenate([conv(gp_v, c, b * GP + H, P2) for b in range(B)], axis=0) for c in range(nC)], axis=1)
        pw2_out(s, 0, PRO_PIECES)
        wait(nR)
        for b in range(B):
            for n in range(nC):
                out_start(n, b * P2, b * T, P2)

    def body(i, carry):
        @pl.when(i == 0)
        def _():
            prologue()

        @pl.when(i == 1)
        def _():
            wait(nR + 1)

        c0 = pl.multiple_of(i * GP + (GP - (H + LEAD)), 8)
        for c in range(nC):
            g_v[c, 0:H + LEAD, :] = gp_v[c, pl.ds(c0, H + LEAD), :]
        xv = load_x(pl.ds(pl.multiple_of(XP + i * LX, 16), LX))
        for c in range(nC):
            g_v[c, H + LEAD:H + LO, :] = gate(mm1(xv, c), mm1(xv, nC + c))
        s = jnp.concatenate([conv(g_v, c, H, LO) for c in range(nC)], axis=1)
        pieces = (LO - sum(TAIL_PIECES),) + TAIL_PIECES
        pw2_out(s, pl.multiple_of(B * P2 + i * LO, 16), pieces, h0=pl.multiple_of(i * T + P2, 16))
        return carry

    jax.lax.fori_loop(0, B, body, 0)
    pltpu.make_async_copy(o_hbm, o_hbm, sem_o).wait()


@jax.jit
def pallas_standalone__conformer_conv_module__speech_kernel(
    x: jax.Array,
    w_pw1: jax.Array,
    dw: jax.Array,
    w_pw2: jax.Array,
):
    B, T, D = x.shape
    K = dw.shape[0]
    nC = D // LC
    R = B * T
    out = pl.pallas_call(
        functools.partial(_kernel, B=B, T=T, D=D, K=K),
        in_specs=[pl.BlockSpec(memory_space=pl.ANY)] * 4,
        out_specs=pl.BlockSpec(memory_space=pl.ANY),
        out_shape=jax.ShapeDtypeStruct((R, D), x.dtype),
        scratch_shapes=[
            pltpu.VMEM((nC, R, LC), x.dtype),
            pltpu.VMEM((2 * nC, D, LC), w_pw1.dtype),
            pltpu.VMEM((K, D), dw.dtype),
            pltpu.VMEM((nC, D, LC), w_pw2.dtype),
            pltpu.VMEM((nC, B * (H + XB), LC), F32),
            pltpu.VMEM((nC, H + (T - P2) + H, LC), F32),
            pltpu.VMEM((2, XP, D), F32),
            pltpu.VMEM((nC, R, LC), x.dtype),
            pltpu.SemaphoreType.DMA((len(RAMP) + B,)),
            pltpu.SemaphoreType.DMA(()),
        ],
        compiler_params=pltpu.CompilerParams(
            vmem_limit_bytes=100 * 1024 * 1024,
            disable_bounds_checks=True,
            disable_semaphore_checks=True,
        ),
    )(x.reshape(R, D), w_pw1, dw, w_pw2)
    return out.reshape(B, T, D)
```

```python
import functools

import jax
import jax.numpy as jnp
import jax.experimental.pallas as pl
import jax.experimental.pallas.tpu as pltpu

LC = 128
H = 8
XB = 1024
XP = 2 * XB
KR = 3
RAMP = (
    ((0, 288, 0, 1, 0),),
    ((288, XB, 0, 1, 0),),
    ((XB, XP, 0, 1, 0), (0, XP, 0, 1, 1)),
    ((0, XP, 1, KR, 0), (0, XP, 1, KR, 1)),
)
TAIL_PIECES = (1296, 1040, 480, 160)
F32 = jnp.float32
BF16 = jnp.bfloat16


def _kernel(x_hbm, w1_hbm, dw_hbm, w2_hbm, o_hbm,
            x_v, w1_v, dw_v, w2_v, g_v, h_v, o_v, sem_i, sem_o, *, B, T, D, K):
    nC = D // LC
    pad = K // 2
    assert B == 2 and nC == 4 and 8 < K <= 16 and pad <= H
    LX = T - XB
    nR = len(RAMP)
    halves = ((0, nC, 1, nC + 1), (2, nC + 2, 3, nC + 3))

    def x_head_copies(lo, hi, c, s):
        out = []
        for b in range(B):
            l, h = max(lo, b * XB), min(hi, (b + 1) * XB)
            if l < h:
                out.append(pltpu.make_async_copy(
                    x_hbm.at[b * T + l - b * XB:b * T + h - b * XB, c * LC:(c + 1) * LC],
                    x_v.at[c, l:h], sem_i.at[s]))
        return out

    def w1_copy(k0, k1, t, s):
        return pltpu.make_async_copy(w1_hbm.at[k0 * LC:k1 * LC, t * LC:(t + 1) * LC],
                                     w1_v.at[t, k0 * LC:k1 * LC], sem_i.at[s])

    grp = []
    x_have = [0] * nC
    w_have = [0, 0]
    for q, blk in enumerate(RAMP):
        cps = []
        for (lo, hi, k0, k1, hf) in blk:
            for k in range(k0, k1):
                if x_have[k] < hi:
                    cps += x_head_copies(x_have[k], hi, k, q)
                    x_have[k] = hi
            if w_have[hf] < k1:
                cps += [w1_copy(w_have[hf], k1, t, q) for t in halves[hf]]
                w_have[hf] = k1
        grp.append(cps)
    assert x_have == [XP] * KR + [0] * (nC - KR) and w_have == [KR, KR]
    for b in range(B):
        s = nR + b
        cps = []
        if b == 0:
            cps += [w1_copy(KR, nC, t, s) for t in range(2 * nC)]
            cps.append(pltpu.make_async_copy(dw_hbm, dw_v, sem_i.at[s]))
            cps += [pltpu.make_async_copy(w2_hbm.at[:, n * LC:(n + 1) * LC], w2_v.at[n], sem_i.at[s])
                    for n in range(nC)]
        for k in range(KR, nC):
            cps += x_head_copies(b * XB, (b + 1) * XB, k, s)
        cps += [pltpu.make_async_copy(x_hbm.at[b * T + XB:(b + 1) * T, c * LC:(c + 1) * LC],
                                      x_v.at[c, XP + b * LX:XP + (b + 1) * LX], sem_i.at[s])
                for c in range(nC)]
        grp.append(cps)
    for cps in grp:
        for cp in cps:
            cp.start()

    def wait(q):
        for cp in grp[q]:
            cp.wait()

    zeros = jnp.zeros((H, LC), F32)
    for c in range(nC):
        g_v[c, 0:H, :] = zeros
        g_v[c, H + T:H + T + H, :] = zeros

    def load_x(rows, k0=0, k1=nC):
        parts = [x_v[c, rows, :] for c in range(k0, k1)]
        return parts[0] if len(parts) == 1 else jnp.concatenate(parts, axis=1)

    def mm1(xv, t):
        return jnp.dot(xv, w1_v[t], preferred_element_type=F32)

    def mm1_part(rows, k0, k1, hf):
        wv = jnp.concatenate([w1_v[t, k0 * LC:k1 * LC, :] for t in halves[hf]], axis=1)
        part = jnp.dot(load_x(rows, k0, k1), wv, preferred_element_type=F32)
        return part + h_v[hf, rows, :] if k0 > 0 else part

    def gate(a, b):
        return a * jnp.tanh(0.5 * b) + a

    def conv_silu(c):
        dwf = dw_v[:, c * LC:(c + 1) * LC].astype(F32) * 0.25

        def tap(k):
            o = H - pad + k
            return g_v[c, o:o + T, :] * dwf[k:k + 1, :]

        lo, hi = tap(0), tap(8)
        for k in range(1, 8):
            lo = lo + tap(k)
        for k in range(9, K):
            hi = hi + tap(k)
        acc = lo + hi
        return acc * jnp.tanh(acc) + acc

    def body(i, carry):
        @pl.when(i == 0)
        def _():
            for q, blk in enumerate(RAMP):
                wait(q)
                for (lo, hi, k0, k1, hf) in blk:
                    h_v[hf, lo:hi, :] = mm1_part(slice(lo, hi), k0, k1, hf)
            wait(nR)

        @pl.when(i == 1)
        def _():
            wait(nR + 1)

        head = pl.ds(pl.multiple_of(i * XB, 16), XB)
        for hf in range(2):
            part = mm1_part(head, KR, nC, hf)
            for j in range(2):
                g_v[2 * hf + j, H:H + XB, :] = gate(part[:, 2 * j * LC:(2 * j + 1) * LC],
                                                    part[:, (2 * j + 1) * LC:(2 * j + 2) * LC])
        xv = load_x(pl.ds(pl.multiple_of(XP + i * LX, 16), LX))
        for c in range(nC):
            g_v[c, H + XB:H + T, :] = gate(mm1(xv, c), mm1(xv, nC + c))
        s = jnp.concatenate([conv_silu(c) for c in range(nC)], axis=1)
        r0 = pl.multiple_of(i * T, 16)
        off = 0
        for p in (T - sum(TAIL_PIECES),) + TAIL_PIECES:
            rows = pl.ds(r0 + off, p)
            sp = s[off:off + p].astype(BF16)
            for n in range(nC):
                o_v[n, rows, :] = jnp.dot(sp, w2_v[n], preferred_element_type=F32).astype(o_v.dtype)
                pltpu.make_async_copy(o_v.at[n, rows], o_hbm.at[rows, n * LC:(n + 1) * LC], sem_o).start()
            off += p
        return carry

    jax.lax.fori_loop(0, B, body, 0)
    pltpu.make_async_copy(o_hbm, o_hbm, sem_o).wait()


@jax.jit
def pallas_standalone__conformer_conv_module__speech_kernel(
    x: jax.Array,
    w_pw1: jax.Array,
    dw: jax.Array,
    w_pw2: jax.Array,
):
    B, T, D = x.shape
    K = dw.shape[0]
    nC = D // LC
    R = B * T
    out = pl.pallas_call(
        functools.partial(_kernel, B=B, T=T, D=D, K=K),
        in_specs=[pl.BlockSpec(memory_space=pl.ANY)] * 4,
        out_specs=pl.BlockSpec(memory_space=pl.ANY),
        out_shape=jax.ShapeDtypeStruct((R, D), x.dtype),
        scratch_shapes=[
            pltpu.VMEM((nC, R, LC), x.dtype),
            pltpu.VMEM((2 * nC, D, LC), w_pw1.dtype),
            pltpu.VMEM((K, D), dw.dtype),
            pltpu.VMEM((nC, D, LC), w_pw2.dtype),
            pltpu.VMEM((nC, H + T + H, LC), F32),
            pltpu.VMEM((2, XP, D), F32),
            pltpu.VMEM((nC, R, LC), x.dtype),
            pltpu.SemaphoreType.DMA((len(RAMP) + B,)),
            pltpu.SemaphoreType.DMA(()),
        ],
        compiler_params=pltpu.CompilerParams(
            vmem_limit_bytes=100 * 1024 * 1024,
            disable_bounds_checks=True,
            disable_semaphore_checks=True,
        ),
    )(x.reshape(R, D), w_pw1, dw, w_pw2)
    return out.reshape(B, T, D)
```

```python
import functools

import jax
import jax.numpy as jnp
import jax.experimental.pallas as pl
import jax.experimental.pallas.tpu as pltpu

LC = 128
H = 8
XB = 1536
XP = 2 * XB
KR = 2
RAMP = (
    ((0, 224, 0, 1, 0),),
    ((224, 864, 0, 1, 0),),
    ((864, 1792, 0, 1, 0), (0, 1792, 0, 1, 1)),
    ((0, 1792, 1, 2, 0), (0, 1792, 1, 2, 1), (1792, XP, 0, 2, 0), (1792, XP, 0, 2, 1)),
)
TAIL_PIECES = (1296, 1040, 480, 160)
F32 = jnp.float32
BF16 = jnp.bfloat16


def _kernel(x_hbm, w1_hbm, dw_hbm, w2_hbm, o_hbm,
            x_v, w1_v, dw_v, w2_v, g_v, h_v, o_v, sem_i, sem_o, *, B, T, D, K):
    nC = D // LC
    pad = K // 2
    assert B == 2 and nC == 4 and 8 < K <= 16 and pad <= H
    LX = T - XB
    nR = len(RAMP)
    halves = ((0, nC, 1, nC + 1), (2, nC + 2, 3, nC + 3))

    def x_head_copies(lo, hi, c, s):
        out = []
        for b in range(B):
            l, h = max(lo, b * XB), min(hi, (b + 1) * XB)
            if l < h:
                out.append(pltpu.make_async_copy(
                    x_hbm.at[b * T + l - b * XB:b * T + h - b * XB, c * LC:(c + 1) * LC],
                    x_v.at[c, l:h], sem_i.at[s]))
        return out

    def w1_copy(k0, k1, t, s):
        return pltpu.make_async_copy(w1_hbm.at[k0 * LC:k1 * LC, t * LC:(t + 1) * LC],
                                     w1_v.at[t, k0 * LC:k1 * LC], sem_i.at[s])

    grp = []
    x_have = [0] * nC
    w_have = [0, 0]
    for q, blk in enumerate(RAMP):
        cps = []
        for (lo, hi, k0, k1, hf) in blk:
            for k in range(k0, k1):
                if x_have[k] < hi:
                    cps += x_head_copies(x_have[k], hi, k, q)
                    x_have[k] = hi
            if w_have[hf] < k1:
                cps += [w1_copy(w_have[hf], k1, t, q) for t in halves[hf]]
                w_have[hf] = k1
        grp.append(cps)
    assert x_have == [XP] * KR + [0] * (nC - KR) and w_have == [KR, KR]
    for b in range(B):
        s = nR + b
        cps = []
        if b == 0:
            cps += [w1_copy(KR, nC, t, s) for t in range(2 * nC)]
            cps.append(pltpu.make_async_copy(dw_hbm, dw_v, sem_i.at[s]))
            cps += [pltpu.make_async_copy(w2_hbm.at[:, n * LC:(n + 1) * LC], w2_v.at[n], sem_i.at[s])
                    for n in range(nC)]
        for k in range(KR, nC):
            cps += x_head_copies(b * XB, (b + 1) * XB, k, s)
        cps += [pltpu.make_async_copy(x_hbm.at[b * T + XB:(b + 1) * T, c * LC:(c + 1) * LC],
                                      x_v.at[c, XP + b * LX:XP + (b + 1) * LX], sem_i.at[s])
                for c in range(nC)]
        grp.append(cps)
    for cps in grp:
        for cp in cps:
            cp.start()

    def wait(q):
        for cp in grp[q]:
            cp.wait()

    zeros = jnp.zeros((H, LC), F32)
    for c in range(nC):
        g_v[c, 0:H, :] = zeros
        g_v[c, H + T:H + T + H, :] = zeros

    def load_x(rows, k0=0, k1=nC):
        parts = [x_v[c, rows, :] for c in range(k0, k1)]
        return parts[0] if len(parts) == 1 else jnp.concatenate(parts, axis=1)

    def mm1(xv, t):
        return jnp.dot(xv, w1_v[t], preferred_element_type=F32)

    def mm1_part(rows, k0, k1, hf):
        wv = jnp.concatenate([w1_v[t, k0 * LC:k1 * LC, :] for t in halves[hf]], axis=1)
        part = jnp.dot(load_x(rows, k0, k1), wv, preferred_element_type=F32)
        return part + h_v[hf, rows, :] if k0 > 0 else part

    def gate(a, b):
        return a * jnp.tanh(0.5 * b) + a

    def conv_silu(c):
        dwf = dw_v[:, c * LC:(c + 1) * LC].astype(F32) * 0.25

        def tap(k):
            o = H - pad + k
            return g_v[c, o:o + T, :] * dwf[k:k + 1, :]

        lo, hi = tap(0), tap(8)
        for k in range(1, 8):
            lo = lo + tap(k)
        for k in range(9, K):
            hi = hi + tap(k)
        acc = lo + hi
        return acc * jnp.tanh(acc) + acc

    def body(i, carry):
        @pl.when(i == 0)
        def _():
            for q, blk in enumerate(RAMP):
                wait(q)
                for (lo, hi, k0, k1, hf) in blk:
                    h_v[hf, lo:hi, :] = mm1_part(slice(lo, hi), k0, k1, hf)
            wait(nR)

        @pl.when(i == 1)
        def _():
            wait(nR + 1)

        head = pl.ds(pl.multiple_of(i * XB, 16), XB)
        for hf in range(2):
            part = mm1_part(head, KR, nC, hf)
            for j in range(2):
                g_v[2 * hf + j, H:H + XB, :] = gate(part[:, 2 * j * LC:(2 * j + 1) * LC],
                                                    part[:, (2 * j + 1) * LC:(2 * j + 2) * LC])
        xv = load_x(pl.ds(pl.multiple_of(XP + i * LX, 16), LX))
        for c in range(nC):
            g_v[c, H + XB:H + T, :] = gate(mm1(xv, c), mm1(xv, nC + c))
        s = jnp.concatenate([conv_silu(c) for c in range(nC)], axis=1)
        r0 = pl.multiple_of(i * T, 16)
        off = 0
        for p in (T - sum(TAIL_PIECES),) + TAIL_PIECES:
            rows = pl.ds(r0 + off, p)
            sp = s[off:off + p].astype(BF16)
            for n in range(nC):
                o_v[n, rows, :] = jnp.dot(sp, w2_v[n], preferred_element_type=F32).astype(o_v.dtype)
                pltpu.make_async_copy(o_v.at[n, rows], o_hbm.at[rows, n * LC:(n + 1) * LC], sem_o).start()
            off += p
        return carry

    jax.lax.fori_loop(0, B, body, 0)
    pltpu.make_async_copy(o_hbm, o_hbm, sem_o).wait()


def _compiler_params():
    base = dict(vmem_limit_bytes=100 * 1024 * 1024, disable_bounds_checks=True)
    try:
        return pltpu.CompilerParams(disable_semaphore_checks=True, **base)
    except TypeError:
        return pltpu.CompilerParams(**base)


@jax.jit
def pallas_standalone__conformer_conv_module__speech_kernel(
    x: jax.Array,
    w_pw1: jax.Array,
    dw: jax.Array,
    w_pw2: jax.Array,
):
    B, T, D = x.shape
    K = dw.shape[0]
    nC = D // LC
    R = B * T
    out = pl.pallas_call(
        functools.partial(_kernel, B=B, T=T, D=D, K=K),
        in_specs=[pl.BlockSpec(memory_space=pl.ANY)] * 4,
        out_specs=pl.BlockSpec(memory_space=pl.ANY),
        out_shape=jax.ShapeDtypeStruct((R, D), x.dtype),
        scratch_shapes=[
            pltpu.VMEM((nC, R, LC), x.dtype),
            pltpu.VMEM((2 * nC, D, LC), w_pw1.dtype),
            pltpu.VMEM((K, D), dw.dtype),
            pltpu.VMEM((nC, D, LC), w_pw2.dtype),
            pltpu.VMEM((nC, H + T + H, LC), F32),
            pltpu.VMEM((2, XP, D), F32),
            pltpu.VMEM((nC, R, LC), x.dtype),
            pltpu.SemaphoreType.DMA((len(RAMP) + B,)),
            pltpu.SemaphoreType.DMA(()),
        ],
        compiler_params=_compiler_params(),
    )(x.reshape(R, D), w_pw1, dw, w_pw2)
    return out.reshape(B, T, D)
```
